```python
import jax
import jax.numpy as jnp

def _softmax(x, axis=-1):
    return jax.nn.softmax(x, axis=axis)
def _gelu(x):
    return jax.nn.gelu(x, approximate=True)
def _silu(x):
    return jax.nn.silu(x)
def _sigmoid(x):
    return jax.nn.sigmoid(x)
def _layernorm(x, axis=-1, eps=1e-5):
    m = jnp.mean(x, axis=axis, keepdims=True)
    v = jnp.var(x, axis=axis, keepdims=True)
    return (x - m) / jnp.sqrt(v + eps)
def _scatter_add(tgt, idx, src, axis=0):
    return tgt.at[idx].add(src)
def _segment_sum(src, seg, n):
    return jax.ops.segment_sum(src, seg, n)
class _Rng:
    def __init__(self, key):
        self._k = key
    def _next(self):
        self._k, sub = jax.random.split(self._k)
        return sub
    def normal(self, shape):
        return jax.random.normal(self._next(), shape, dtype=jnp.bfloat16)
    def randint(self, lo, hi, shape):
        return jax.random.randint(self._next(), shape, lo, hi, dtype=jnp.int32)
    def uniform(self, shape, lo=0.0, hi=1.0):
        return jax.random.uniform(self._next(), shape, jnp.bfloat16, lo, hi)
    def permutation(self, n):
        return jax.random.permutation(self._next(), n)


kernel_name = 'standalone__depthwise_separable__vision'

def setup_inputs():
    _rng = _Rng(jax.random.key(int.from_bytes(__import__("os").urandom(4), "little")))
    _w = (lambda a: (lambda t: t.astype(jnp.bfloat16) if jnp.issubdtype(t.dtype, jnp.floating) else t)(jnp.asarray(a)))
    H = W = 384
    C = 384
    k = 1
    return {
        "x": _w((lambda *s: _rng.normal(s) * 0.05)(1, H, W, C)),
        "dw": _w((lambda *s: _rng.normal(s) * 0.05)(k, k, C)),
        "pw": _w((lambda *s: _rng.normal(s) * 0.05)(C, C)),
    }

def reference(x, dw, pw):
    B, H, W, C = x.shape
    k = dw.shape[0]
    pad = k // 2
    xp = jnp.pad(x, ((0,0),(pad,pad),(pad,pad),(0,0)))
    out = jnp.zeros_like(x)
    for i in range(k):
        for j in range(k):
            out = out + xp[:, i:i+H, j:j+W, :] * dw[i, j][None, None, None, :]
    return jnp.einsum('bhwc,cd->bhwd', out, pw)
```

```python
import jax
import jax.numpy as jnp
from jax import lax
import jax.experimental.pallas as pl
import jax.experimental.pallas.tpu as pltpu

_S = 6
_U = 96
_RW = 48
_NR = 16
_TAIL = 48
_LEAD = 4


def _kernel(x_hbm, dw_hbm, pw_hbm, o_hbm, buf, dw_v, pw_v, rsem, wsem, psem):
    S, L, C = buf.shape
    n = L // _U
    n1 = n // 2
    upc = n // _NR
    t = upc * _U

    def last_read(c):
        rows = pl.ds(c * t, t - _TAIL) if c == _NR - 1 else pl.ds(L - _TAIL, _TAIL)
        return pltpu.make_async_copy(x_hbm.at[:, rows], buf.at[:, rows], rsem.at[c])

    def start_read(c, _):
        rows = pl.ds(pl.multiple_of(c * t, t), t)
        pltpu.make_async_copy(x_hbm.at[:, rows], buf.at[:, rows], rsem.at[c]).start()

    def wait_read(c):
        v = buf.at[:, pl.ds(0, t)]
        pltpu.make_async_copy(v, v, rsem.at[c]).wait()

    def compute(u):
        rows = pl.ds(pl.multiple_of(u * _U, _U), _U)
        xv = buf[:, rows].reshape(S * _U, C)
        xv = (xv.astype(jnp.float32) * dw_v[...].astype(jnp.float32)).astype(buf.dtype)
        y = jnp.dot(xv, pw_v[...], preferred_element_type=jnp.float32)
        buf[:, rows] = y.astype(buf.dtype).reshape(S, _U, C)

    def write(u):
        for h in range(_U // _RW):
            rows = pl.ds(pl.multiple_of(u * _U + h * _RW, _RW), _RW)
            pltpu.make_async_copy(buf.at[:, rows], o_hbm.at[:, rows], wsem).start()

    pw_copy = pltpu.make_async_copy(pw_hbm, pw_v, psem.at[0])
    dw_copy = pltpu.make_async_copy(dw_hbm, dw_v, psem.at[1])
    pw_copy.start()
    dw_copy.start()
    lax.fori_loop(0, _NR - 1, start_read, None)
    last_read(_NR - 1).start()
    pw_copy.wait()
    dw_copy.wait()
    last_read(_NR).start()

    def step(i, _):
        @pl.when((i < n1) & (i % upc == 0))
        def _():
            wait_read(i // upc)

        @pl.when(i == n1)
        def _():
            for c in range(n1 // upc, _NR - 1):
                wait_read(c)
            last_read(_NR - 1).wait()
            for u in range(_LEAD):
                write(u)
            last_read(_NR).wait()

        compute(i)

        @pl.when(i >= n1)
        def _():
            lo = jnp.minimum(_LEAD + 2 * (i - n1), i)
            hi = jnp.minimum(_LEAD + 2 * (i - n1) + 2, i + 1)

            @pl.when(lo < hi)
            def _():
                write(lo)

            @pl.when(lo + 1 < hi)
            def _():
                write(lo + 1)

    lax.fori_loop(0, n, step, None)
    pltpu.make_async_copy(buf, buf, wsem).wait()


@jax.jit
def pallas_standalone__depthwise_separable__vision_kernel(
    x: jax.Array,
    dw: jax.Array,
    pw: jax.Array,
):
    B, H, W, C = x.shape
    assert dw.shape == (1, 1, C) and pw.shape == (C, C)
    shape = (_S, B * H * W // _S, C)
    assert shape[1] % (2 * _U * _NR) == 0
    out = pl.pallas_call(
        _kernel,
        in_specs=[pl.BlockSpec(memory_space=pl.ANY)] * 3,
        out_specs=pl.BlockSpec(memory_space=pl.ANY),
        out_shape=jax.ShapeDtypeStruct(shape, x.dtype),
        scratch_shapes=[
            pltpu.VMEM(shape, x.dtype),
            pltpu.VMEM((1, C), dw.dtype),
            pltpu.VMEM((C, C), pw.dtype),
            pltpu.SemaphoreType.DMA((_NR + 1,)),
            pltpu.SemaphoreType.DMA(()),
            pltpu.SemaphoreType.DMA((2,)),
        ],
        compiler_params=pltpu.CompilerParams(vmem_limit_bytes=120 * 1024 * 1024),
    )(x.reshape(shape), dw.reshape(1, C), pw)
    return out.reshape(B, H, W, C)
```

```python
import jax
import jax.numpy as jnp
from jax import lax
import jax.experimental.pallas as pl
import jax.experimental.pallas.tpu as pltpu

_STREAMS = 8
_READ_STREAMS = 2
_READ_ROWS = 32
_GROUP = 192
_AHEAD = 2
_TAIL = 128
_MICRO = 8
_UNIT = 96
_WRITE_ROWS = 48
_LEAD = 6
_SLOTS = _AHEAD + 1


def _kernel(x_hbm, dw_hbm, pw_hbm, o_hbm, buf, dw_v, pw_v, rsem, wsem, psem):
    S, L, C = buf.shape
    n_groups = L // _GROUP
    n_units = L // _UNIT
    pairs = [
        (row, s)
        for row in range(0, _GROUP, _READ_ROWS)
        for s in range(0, S, 2 * _READ_STREAMS)
    ]
    assert len(pairs) * _MICRO == _UNIT

    def start_read_pair(row, s, slot):
        for priority in range(2):
            idx = (pl.ds(s + priority * _READ_STREAMS, _READ_STREAMS), pl.ds(row, _READ_ROWS))
            copy = pltpu.make_async_copy(x_hbm.at[idx], buf.at[idx], rsem.at[slot])
            copy.start(priority=priority)

    def wait_reads(row, n_rows, slot):
        idx = (slice(None), pl.ds(row, n_rows))
        pltpu.make_async_copy(x_hbm.at[idx], buf.at[idx], rsem.at[slot]).wait()

    def transform(row, n_rows):
        x = buf[:, pl.ds(row, n_rows)].reshape(S * n_rows, C)
        x = (x.astype(jnp.float32) * dw_v[...].astype(jnp.float32)).astype(buf.dtype)
        y = jnp.dot(x, pw_v[...], preferred_element_type=jnp.float32)
        return y.astype(buf.dtype).reshape(S, n_rows, C)

    def start_writes(unit):
        for row in range(0, _UNIT, _WRITE_ROWS):
            rows = pl.ds(pl.multiple_of(unit * _UNIT + row, _WRITE_ROWS), _WRITE_ROWS)
            pltpu.make_async_copy(buf.at[:, rows], o_hbm.at[:, rows], wsem).start()

    pw_copy = pltpu.make_async_copy(pw_hbm, pw_v, psem.at[0])
    dw_copy = pltpu.make_async_copy(dw_hbm, dw_v, psem.at[1])
    pw_copy.start()
    dw_copy.start(priority=1)

    def first_groups(g, _):
        for row, s in pairs:
            start_read_pair(pl.multiple_of(g * _GROUP + row, _READ_ROWS), s, g)

    lax.fori_loop(0, _AHEAD, first_groups, None)
    pw_copy.wait()
    dw_copy.wait()

    def read_step(g, slot):
        next_slot = jnp.where(slot + 1 == _SLOTS, 0, slot + 1)
        wait_reads(pl.multiple_of((g - _AHEAD) * _GROUP, _GROUP), _GROUP, next_slot)
        pending = None
        for k, (row, s) in enumerate(pairs):
            start_read_pair(pl.multiple_of(g * _GROUP + row, _READ_ROWS), s, slot)
            at = pl.multiple_of((g - _AHEAD) * _UNIT + k * _MICRO, _MICRO)
            y = transform(at, _MICRO)
            if pending is not None:
                buf[:, pl.ds(pending[0], _MICRO)] = pending[1]
            pending = (at, y)
        buf[:, pl.ds(pending[0], _MICRO)] = pending[1]
        return next_slot

    last = n_groups - 1
    lax.fori_loop(_AHEAD, last, read_step, jnp.int32(_AHEAD))
    for row, s in pairs:
        slot = last % _SLOTS if row < _GROUP - _TAIL else _SLOTS
        start_read_pair(last * _GROUP + row, s, slot)
    for g in range(last - _AHEAD, last):
        wait_reads(g * _GROUP, _GROUP, g % _SLOTS)
    wait_reads(last * _GROUP, _GROUP - _TAIL, last % _SLOTS)

    done = last - _AHEAD
    assert _LEAD <= done and _LEAD + 2 * (n_units - done) >= n_units
    for unit in range(_LEAD):
        start_writes(unit)
    wait_reads(L - _TAIL, _TAIL, _SLOTS)

    def write_step(i, written):
        at = pl.multiple_of(i * _UNIT, _UNIT)
        buf[:, pl.ds(at, _UNIT)] = transform(at, _UNIT)
        start_writes(written)

        @pl.when(written < i)
        def _():
            start_writes(written + 1)

        return jnp.minimum(written + 2, i + 1)

    lax.fori_loop(done, n_units, write_step, jnp.int32(_LEAD))
    pltpu.make_async_copy(buf, o_hbm, wsem).wait()


@jax.jit
def pallas_standalone__depthwise_separable__vision_kernel(
    x: jax.Array,
    dw: jax.Array,
    pw: jax.Array,
):
    B, H, W, C = x.shape
    assert dw.shape == (1, 1, C) and pw.shape == (C, C)
    assert (B * H * W) % (_STREAMS * _GROUP) == 0
    shape = (_STREAMS, B * H * W // _STREAMS, C)
    out = pl.pallas_call(
        _kernel,
        in_specs=[pl.BlockSpec(memory_space=pl.ANY)] * 3,
        out_specs=pl.BlockSpec(memory_space=pl.ANY),
        out_shape=jax.ShapeDtypeStruct(shape, x.dtype),
        scratch_shapes=[
            pltpu.VMEM(shape, x.dtype),
            pltpu.VMEM((1, C), dw.dtype),
            pltpu.VMEM((C, C), pw.dtype),
            pltpu.SemaphoreType.DMA((_SLOTS + 1,)),
            pltpu.SemaphoreType.DMA(()),
            pltpu.SemaphoreType.DMA((2,)),
        ],
        compiler_params=pltpu.CompilerParams(vmem_limit_bytes=120 * 1024 * 1024),
    )(x.reshape(shape), dw.reshape(1, C), pw)
    return out.reshape(B, H, W, C)
```
